```python
import os as _os
_os.environ.setdefault("JAX_PLATFORMS", "cpu")
import jax
import jax.numpy as jnp

def _softmax(x, axis=-1):
    return jax.nn.softmax(x, axis=axis)
def _gelu(x):
    return jax.nn.gelu(x, approximate=True)
def _silu(x):
    return jax.nn.silu(x)
def _sigmoid(x):
    return jax.nn.sigmoid(x)
def _layernorm(x, axis=-1, eps=1e-5):
    m = jnp.mean(x, axis=axis, keepdims=True)
    v = jnp.var(x, axis=axis, keepdims=True)
    return (x - m) / jnp.sqrt(v + eps)
def _scatter_add(tgt, idx, src, axis=0):
    return tgt.at[idx].add(src)
def _segment_sum(src, seg, n):
    return jax.ops.segment_sum(src, seg, n)
class _Rng:
    def __init__(self, key):
        self._k = key
    def _next(self):
        self._k, sub = jax.random.split(self._k)
        return sub
    def normal(self, shape):
        return jax.random.normal(self._next(), shape, dtype=jnp.bfloat16)
    def randint(self, lo, hi, shape):
        return jax.random.randint(self._next(), shape, lo, hi, dtype=jnp.int32)
    def uniform(self, shape, lo=0.0, hi=1.0):
        return jax.random.uniform(self._next(), shape, jnp.bfloat16, lo, hi)
    def permutation(self, n):
        return jax.random.permutation(self._next(), n)


kernel_name = 'gated_mix__ssm_conv_s5__glu_gated_geglu__prompt'

def setup_inputs():
    _rng = _Rng(jax.random.key(int.from_bytes(__import__("os").urandom(4), "little")))
    _w = (lambda a: (lambda t: t.astype(jnp.bfloat16) if jnp.issubdtype(t.dtype, jnp.floating) else t)(jnp.asarray(a)))
    def _A_setup():
        B, S, D = 1, 2048, 1024
        P = D
        Lambda_re = -0.5 * jnp.exp((lambda *s: _rng.normal(s) * 0.4)(P))
        Lambda_im = (lambda *s: _rng.normal(s) * 0.4)(P) * 1.0
        B_re = (lambda *s: _rng.normal(s) * 0.4)(P, D) * (D ** -0.5)
        B_im = (lambda *s: _rng.normal(s) * 0.4)(P, D) * (D ** -0.5)
        C_re = (lambda *s: _rng.normal(s) * 0.4)(D, P) * (P ** -0.5)
        C_im = (lambda *s: _rng.normal(s) * 0.4)(D, P) * (P ** -0.5)
        log_dt = (lambda *s: _rng.normal(s) * 0.4)(P) * 0.3 - 2.0
        Dskip = (lambda *s: _rng.normal(s) * 0.4)(D)
        return {
            "x": _w((lambda *s: _rng.normal(s) * 0.05)(B, S, D)),
            "Lambda_re": _w(Lambda_re),
            "Lambda_im": _w(Lambda_im),
            "B_re": _w(B_re),
            "B_im": _w(B_im),
            "C_re": _w(C_re),
            "C_im": _w(C_im),
            "log_dt": _w(log_dt),
            "Dskip": _w(Dskip),
        }
    _A_in = _A_setup()

    def _B_setup():
        B, S, Dm, Df = 1, 2048, 1024, 3584
        return {
            "x": _w((lambda *s: _rng.normal(s) * 0.05)(B, S, Dm)),
            "w_gate": _w((lambda *s: _rng.normal(s) * 1.6)(Dm, Df) * (Dm ** -0.5)),
            "w_up": _w((lambda *s: _rng.normal(s) * 1.6)(Dm, Df) * (Dm ** -0.5)),
            "w_down": _w((lambda *s: _rng.normal(s) * 1.6)(Df, Dm) * (Df ** -0.5)),
        }
    _B_in = _B_setup()

    return {
        "A_x": _A_in["x"],
        "A_Lambda_re": _A_in["Lambda_re"],
        "A_Lambda_im": _A_in["Lambda_im"],
        "A_B_re": _A_in["B_re"],
        "A_B_im": _A_in["B_im"],
        "A_C_re": _A_in["C_re"],
        "A_C_im": _A_in["C_im"],
        "A_log_dt": _A_in["log_dt"],
        "A_Dskip": _A_in["Dskip"],
        "B_x": _B_in["x"],
        "B_w_gate": _B_in["w_gate"],
        "B_w_up": _B_in["w_up"],
        "B_w_down": _B_in["w_down"],
        "gate_w": _w((lambda *s: _rng.normal(s) * 0.05)(1024) * 16.0),
    }

def reference(A_x, A_Lambda_re, A_Lambda_im, A_B_re, A_B_im, A_C_re, A_C_im, A_log_dt, A_Dskip, B_x, B_w_gate, B_w_up, B_w_down, gate_w):
    def _A_ref(x, Lambda_re, Lambda_im, B_re, B_im, C_re, C_im, log_dt, Dskip):
        Bsz, L, H = x.shape
        Lam = Lambda_re + 1j * Lambda_im
        Bmat = B_re + 1j * B_im
        Cmat = C_re + 1j * C_im
        dt = jnp.exp(log_dt)
        Lam_bar = jnp.exp(dt * Lam)
        B_bar = ((Lam_bar - 1.0) / Lam)[:, None] * Bmat
        Bu = jnp.einsum("bld,pd->blp", x + 0j, B_bar)
        h = jnp.zeros_like(Bu[:, 0, :])
        hs = []
        for t in range(L):
            h = Lam_bar[None, :] * h + Bu[:, t, :]
            hs.append(h)
        hseq = jnp.stack(hs, 1)
        y = 2.0 * jnp.einsum("blp,dp->bld", hseq, Cmat).real + x * Dskip[None, None, :]
        return y

    def _B_ref(x, w_gate, w_up, w_down):
        g = jnp.einsum("bsd,df->bsf", x, w_gate)
        u = jnp.einsum("bsd,df->bsf", x, w_up)
        h = _gelu(g) * u
        return jnp.einsum("bsf,fd->bsd", h, w_down)

    x = A_x
    g = _sigmoid((x * gate_w).sum(-1, keepdims=True))
    a = _A_ref(x, A_Lambda_re, A_Lambda_im, A_B_re, A_B_im, A_C_re, A_C_im, A_log_dt, A_Dskip)
    b = _B_ref(x, B_w_gate, B_w_up, B_w_down)
    return g * a + (1 - g) * b
```

```python
import functools

import jax
import jax.numpy as jnp
from jax import lax
import jax.experimental.pallas as pl
import jax.experimental.pallas.tpu as pltpu

F32 = jnp.float32
BF16 = jnp.bfloat16

TM = 512
FC = 512
NSEG = 8


def _rb(v):
    return v.astype(BF16).astype(F32)


def _nt(a, b):
    return lax.dot_general(a, b, (((1,), (1,)), ((), ())),
                           preferred_element_type=F32)


def _kernel(x_ref, lre_ref, lim_ref, ldt_ref, dsk_ref, gw_ref,
            bre_hbm, bim_hbm, cre_hbm, cim_hbm, wg_hbm, wu_hbm, wd_hbm,
            o_ref,
            b_vm, c_vm, wg_vm, wu_vm, wd_vm, sems,
            bu_ref, cst_ref, st_ref, acc_ref, *, P, D, NC):
    step = pl.program_id(0)
    L = TM // NSEG

    def b_copies():
        return (pltpu.make_async_copy(bre_hbm, b_vm.at[pl.ds(0, P)], sems.at[0]),
                pltpu.make_async_copy(bim_hbm, b_vm.at[pl.ds(P, P)], sems.at[1]))

    def c_copies():
        return (pltpu.make_async_copy(cre_hbm, c_vm.at[:, pl.ds(0, P)], sems.at[2]),
                pltpu.make_async_copy(cim_hbm, c_vm.at[:, pl.ds(P, P)], sems.at[3]))

    def w_copies(c):
        off = pl.multiple_of(c * FC, FC)
        return (pltpu.make_async_copy(wg_hbm.at[:, pl.ds(off, FC)], wg_vm.at[c], sems.at[4 + 3 * c]),
                pltpu.make_async_copy(wu_hbm.at[:, pl.ds(off, FC)], wu_vm.at[c], sems.at[5 + 3 * c]),
                pltpu.make_async_copy(wd_hbm.at[pl.ds(off, FC), :], wd_vm.at[c], sems.at[6 + 3 * c]))

    @pl.when(step == 0)
    def _init():
        for cp in b_copies():
            cp.start()
        for c in range(NC):
            for cp in w_copies(c):
                cp.start()
        for cp in c_copies():
            cp.start()
        lre = lre_ref[...].astype(F32)
        lim = lim_ref[...].astype(F32)
        dt = _rb(jnp.exp(ldt_ref[...].astype(F32)))
        zr = dt * lre
        zi = dt * lim

        def cexp(k):
            m = jnp.exp(zr * k)
            return m * jnp.cos(zi * k), m * jnp.sin(zi * k)

        ar, ai = cexp(1.0)
        nr = ar - 1.0
        ni = ai
        den = lre * lre + lim * lim
        cr = (nr * lre + ni * lim) / den
        ci = (ni * lre - nr * lim) / den
        pr, pi_ = ar, ai
        k = 1
        while k < L:
            pr, pi_ = pr * pr - pi_ * pi_, 2.0 * pr * pi_
            k *= 2
        cst_ref[0] = jnp.broadcast_to(ar, (8, P))
        cst_ref[1] = jnp.broadcast_to(ai, (8, P))
        cst_ref[2] = jnp.broadcast_to(cr, (8, P))
        cst_ref[3] = jnp.broadcast_to(ci, (8, P))
        cst_ref[4] = jnp.broadcast_to(pr, (8, P))
        cst_ref[5] = jnp.broadcast_to(pi_, (8, P))
        st_ref[...] = jnp.zeros_like(st_ref)
        for cp in b_copies():
            cp.wait()

    xb = x_ref[...]

    NT = P // 128
    v = _nt(xb, b_vm[...])
    for j in range(NT):
        sl = slice(j * 128, (j + 1) * 128)
        vr = v[:, j * 128:(j + 1) * 128]
        vi = v[:, P + j * 128:P + (j + 1) * 128]
        cr = cst_ref[2, 0:1, sl]
        ci = cst_ref[3, 0:1, sl]
        bu_ref[j] = cr * vr - ci * vi
        bu_ref[NT + j] = cr * vi + ci * vr

    def scan_body(store):
        def body(i, carry):
            hr, hi = carry
            nr, ni = [], []
            for j in range(NT):
                ar = cst_ref[0, :, j * 128:(j + 1) * 128]
                ai = cst_ref[1, :, j * 128:(j + 1) * 128]
                ur = bu_ref[j, pl.ds(i, NSEG, stride=L), :]
                ui = bu_ref[NT + j, pl.ds(i, NSEG, stride=L), :]
                nhr = ar * hr[j] - ai * hi[j] + ur
                nhi = ar * hi[j] + ai * hr[j] + ui
                if store:
                    bu_ref[j, pl.ds(i, NSEG, stride=L), :] = nhr
                    bu_ref[NT + j, pl.ds(i, NSEG, stride=L), :] = nhi
                nr.append(nhr)
                ni.append(nhi)
            return tuple(nr), tuple(ni)
        return body

    z = tuple(jnp.zeros((NSEG, 128), F32) for _ in range(NT))
    er, ei = lax.fori_loop(0, L, scan_body(False), (z, z))
    er = jnp.concatenate(er, axis=1)
    ei = jnp.concatenate(ei, axis=1)
    pr = cst_ref[4, 0:1, :]
    pi_ = cst_ref[5, 0:1, :]
    cur_r = st_ref[0:1, pl.ds(0, P)]
    cur_i = st_ref[0:1, pl.ds(P, P)]
    rows_r, rows_i = [cur_r], [cur_i]
    for s in range(NSEG - 1):
        cur_r, cur_i = (er[s:s + 1] + pr * cur_r - pi_ * cur_i,
                        ei[s:s + 1] + pr * cur_i + pi_ * cur_r)
        rows_r.append(cur_r)
        rows_i.append(cur_i)
    h0r = jnp.concatenate(rows_r, axis=0)
    h0i = jnp.concatenate(rows_i, axis=0)
    h0r = tuple(h0r[:, j * 128:(j + 1) * 128] for j in range(NT))
    h0i = tuple(h0i[:, j * 128:(j + 1) * 128] for j in range(NT))
    fr, fi = lax.fori_loop(0, L, scan_body(True), (h0r, h0i))
    st_ref[0:1, pl.ds(0, P)] = jnp.concatenate(fr, axis=1)[NSEG - 1:NSEG]
    st_ref[0:1, pl.ds(P, P)] = jnp.concatenate(fi, axis=1)[NSEG - 1:NSEG]

    acc_ref[...] = jnp.zeros_like(acc_ref)

    def chunk(c, carry):
        @pl.when(step == 0)
        def _():
            for cp in w_copies(c):
                cp.wait()
        g = _rb(jnp.dot(xb, wg_vm[c], preferred_element_type=F32))
        u = _rb(jnp.dot(xb, wu_vm[c], preferred_element_type=F32))
        hh = (_rb(jax.nn.gelu(g, approximate=True)) * u).astype(BF16)
        acc_ref[...] += jnp.dot(hh, wd_vm[c], preferred_element_type=F32)
        return carry

    lax.fori_loop(0, NC, chunk, 0)

    @pl.when(step == 0)
    def _():
        for cp in c_copies():
            cp.wait()

    hcat = jnp.concatenate([bu_ref[j].astype(BF16) for j in range(NT)]
                           + [(-bu_ref[NT + j]).astype(BF16) for j in range(NT)], axis=1)
    y = _nt(hcat, c_vm[...])

    xf = xb.astype(F32)
    a = 2.0 * y + _rb(xf * dsk_ref[...].astype(F32))
    logit = _rb(jnp.sum(_rb(xf * gw_ref[...].astype(F32)), axis=-1, keepdims=True))
    g = _rb(jax.nn.sigmoid(logit))
    b = _rb(acc_ref[...])
    o_ref[...] = g * a + _rb(_rb(1.0 - g) * b)


@jax.jit
def pallas_gated_mix__ssm_conv_s5__glu_gated_geglu__prompt_kernel(
    A_x, A_Lambda_re, A_Lambda_im, A_B_re, A_B_im, A_C_re, A_C_im, A_log_dt,
    A_Dskip, B_x, B_w_gate, B_w_up, B_w_down, gate_w,
):
    Bsz, S, D = A_x.shape
    P = A_Lambda_re.shape[0]
    Df = B_w_gate.shape[1]
    assert Bsz == 1 and S % TM == 0 and Df % FC == 0
    NC = Df // FC

    x2 = A_x.reshape(S, D)
    row = lambda a: a.reshape(1, -1)

    vec_spec = lambda n: pl.BlockSpec((1, n), lambda i: (0, 0))
    any_spec = pl.BlockSpec(memory_space=pl.ANY)

    out = pl.pallas_call(
        functools.partial(_kernel, P=P, D=D, NC=NC),
        grid=(S // TM,),
        in_specs=[pl.BlockSpec((TM, D), lambda i: (i, 0)),
                  vec_spec(P), vec_spec(P), vec_spec(P), vec_spec(D), vec_spec(D)]
                 + [any_spec] * 7,
        out_specs=pl.BlockSpec((TM, D), lambda i: (i, 0)),
        out_shape=jax.ShapeDtypeStruct((S, D), F32),
        scratch_shapes=[
            pltpu.VMEM((2 * P, D), BF16),
            pltpu.VMEM((D, 2 * P), BF16),
            pltpu.VMEM((NC, D, FC), BF16),
            pltpu.VMEM((NC, D, FC), BF16),
            pltpu.VMEM((NC, FC, D), BF16),
            pltpu.SemaphoreType.DMA((4 + 3 * NC,)),
            pltpu.VMEM((2 * P // 128, TM, 128), F32),
            pltpu.VMEM((6, 8, P), F32),
            pltpu.VMEM((8, 2 * P), F32),
            pltpu.VMEM((TM, D), F32),
        ],
        compiler_params=pltpu.CompilerParams(
            dimension_semantics=("arbitrary",),
            vmem_limit_bytes=100 * 1024 * 1024,
        ),
    )(x2, row(A_Lambda_re), row(A_Lambda_im), row(A_log_dt), row(A_Dskip), row(gate_w),
      A_B_re, A_B_im, A_C_re, A_C_im, B_w_gate, B_w_up, B_w_down)
    return out.reshape(Bsz, S, D)
```

```python
import functools

import jax
import jax.numpy as jnp
from jax import lax
import jax.experimental.pallas as pl
import jax.experimental.pallas.tpu as pltpu

F32 = jnp.float32
BF16 = jnp.bfloat16

TM = 512
FC = 896
SL = 128
NS = TM // SL
NH = 4
NQ = 4


def _rb(v):
    return v.astype(BF16).astype(F32)


def _nt(a, b):
    return lax.dot_general(a, b, (((1,), (1,)), ((), ())),
                           preferred_element_type=F32)


def _kernel(x_ref, lre_ref, lim_ref, ldt_ref, dsk_ref, gw_ref,
            bre_hbm, bim_hbm, cre_hbm, cim_hbm, wg_hbm, wu_hbm, wd_hbm,
            o_hbm,
            b_vm, c_vm, wg_vm, wu_vm, wd_vm, sems, bsems, osems,
            bu_ref, cst_ref, st_ref, acc_ref, obuf, *, P, D, NC, NB):
    step = pl.program_id(0)
    H = P // NQ

    def b_copy(q):
        src = bre_hbm if q % 2 == 0 else bim_hbm
        grp = q // 2
        return pltpu.make_async_copy(src.at[pl.ds(grp * H, H)],
                                     b_vm.at[pl.ds((q % 2) * P + grp * H, H)], bsems.at[q])

    def c_copies():
        return (pltpu.make_async_copy(cre_hbm, c_vm.at[:, pl.ds(0, P)], sems.at[0]),
                pltpu.make_async_copy(cim_hbm, c_vm.at[:, pl.ds(P, P)], sems.at[1]))

    def w_copies(c):
        off = pl.multiple_of(c * FC, FC)
        return (pltpu.make_async_copy(wg_hbm.at[:, pl.ds(off, FC)], wg_vm.at[c], sems.at[2 + 3 * c]),
                pltpu.make_async_copy(wu_hbm.at[:, pl.ds(off, FC)], wu_vm.at[c], sems.at[3 + 3 * c]),
                pltpu.make_async_copy(wd_hbm.at[pl.ds(off, FC), :], wd_vm.at[c], sems.at[4 + 3 * c]))

    RH = TM // NH

    def o_copy(blk, hf):
        slot = blk % 2
        return pltpu.make_async_copy(obuf.at[slot, pl.ds(hf * RH, RH)],
                                     o_hbm.at[pl.ds(blk * TM + hf * RH, RH)],
                                     osems.at[slot * NH + hf])

    @pl.when(step >= 2)
    def _():
        for hf in range(NH):
            o_copy(step - 2, hf).wait()

    @pl.when(step == 0)
    def _init():
        for q in range(2 * NQ):
            b_copy(q).start()
        lre = lre_ref[...].astype(F32).reshape(1, P)
        lim = lim_ref[...].astype(F32).reshape(1, P)
        dt = _rb(jnp.exp(ldt_ref[...].astype(F32).reshape(1, P)))
        zr = dt * lre
        zi = dt * lim
        m = jnp.exp(zr)
        ar, ai = m * jnp.cos(zi), m * jnp.sin(zi)
        nr = ar - 1.0
        ni = ai
        den = lre * lre + lim * lim
        cr = (nr * lre + ni * lim) / den
        ci = (ni * lre - nr * lim) / den
        cst_ref[0] = jnp.broadcast_to(cr, (8, P))
        cst_ref[1] = jnp.broadcast_to(ci, (8, P))
        pw = [(ar, ai)]
        for _ in range(7):
            qr, qi = pw[-1]
            pw.append((qr * ar - qi * ai, qr * ai + qi * ar))
        row = lax.broadcasted_iota(jnp.int32, (8, P), 0)
        for n, d in enumerate((1, 2, 4)):
            cst_ref[2 + 2 * n] = jnp.where(row >= d, jnp.broadcast_to(pw[d - 1][0], (8, P)), 0.0)
            cst_ref[3 + 2 * n] = jnp.where(row >= d, jnp.broadcast_to(pw[d - 1][1], (8, P)), 0.0)
        cst_ref[8] = jnp.concatenate([p[0] for p in pw], axis=0)
        cst_ref[9] = jnp.concatenate([p[1] for p in pw], axis=0)
        st_ref[...] = jnp.zeros_like(st_ref)

    xb = x_ref[...]

    for q in range(NQ):
        @pl.when(step == 0)
        def _():
            b_copy(2 * q).wait()
            b_copy(2 * q + 1).wait()
            for cp in w_copies(q):
                cp.start()
            if q == NQ - 1:
                for cp in c_copies():
                    cp.start()
        vr = _nt(xb, b_vm[pl.ds(q * H, H), :])
        vi = _nt(xb, b_vm[pl.ds(P + q * H, H), :])
        cr = cst_ref[0, 0:1, pl.ds(q * H, H)]
        ci = cst_ref[1, 0:1, pl.ds(q * H, H)]
        bu_ref[:, pl.ds(q * H, H)] = cr * vr - ci * vi
        bu_ref[:, pl.ds(P + q * H, H)] = cr * vi + ci * vr

    def slab_scan(sb):
        base = pl.multiple_of(sb * SL, SL)
        srow = lax.broadcasted_iota(jnp.int32, (8, 128), 0)
        for j in range(P // 128):
            lo = j * 128
            cd = [(cst_ref[2 + 2 * n, :, pl.ds(lo, 128)], cst_ref[3 + 2 * n, :, pl.ds(lo, 128)])
                  for n in range(3)]
            pwr = cst_ref[8, :, pl.ds(lo, 128)]
            pwi = cst_ref[9, :, pl.ds(lo, 128)]
            hr = st_ref[0:1, pl.ds(lo, 128)]
            hi = st_ref[0:1, pl.ds(P + lo, 128)]
            for k in range(SL // 8):
                rows = pl.ds(pl.multiple_of(base + k * 8, 8), 8)
                ur = bu_ref[rows, pl.ds(lo, 128)]
                ui = bu_ref[rows, pl.ds(P + lo, 128)]
                for n, d in enumerate((1, 2, 4)):
                    sr = jnp.where(srow >= d, pltpu.roll(ur, d, 0), 0.0)
                    si = jnp.where(srow >= d, pltpu.roll(ui, d, 0), 0.0)
                    cdr, cdi = cd[n]
                    ur, ui = ur + cdr * sr - cdi * si, ui + cdr * si + cdi * sr
                br = jnp.broadcast_to(hr, (8, 128))
                bi = jnp.broadcast_to(hi, (8, 128))
                ur, ui = ur + pwr * br - pwi * bi, ui + pwr * bi + pwi * br
                bu_ref[rows, pl.ds(lo, 128)] = ur
                bu_ref[rows, pl.ds(P + lo, 128)] = ui
                hr = ur[7:8]
                hi = ui[7:8]
            st_ref[0:1, pl.ds(lo, 128)] = hr
            st_ref[0:1, pl.ds(P + lo, 128)] = hi

    acc_ref[...] = jnp.zeros_like(acc_ref)

    def chunk(c, carry):
        @pl.when(step == 0)
        def _():
            for cp in w_copies(c):
                cp.wait()
        slab_scan(c)
        g = _rb(jnp.dot(xb, wg_vm[c], preferred_element_type=F32))
        u = _rb(jnp.dot(xb, wu_vm[c], preferred_element_type=F32))
        hh = (_rb(jax.nn.gelu(g, approximate=True)) * u).astype(BF16)
        acc_ref[...] += jnp.dot(hh, wd_vm[c], preferred_element_type=F32)
        return carry

    lax.fori_loop(0, NC, chunk, 0)

    @pl.when(step == 0)
    def _():
        for cp in c_copies():
            cp.wait()

    for hf in range(NH):
        rows = pl.ds(hf * RH, RH)
        hcat = jnp.concatenate([bu_ref[rows, pl.ds(0, P)], -bu_ref[rows, pl.ds(P, P)]],
                               axis=1).astype(BF16)
        y = _nt(hcat, c_vm[...])
        xf = x_ref[rows, :].astype(F32)
        a = 2.0 * y + _rb(xf * dsk_ref[...].astype(F32).reshape(1, D))
        logit = _rb(jnp.sum(_rb(xf * gw_ref[...].astype(F32).reshape(1, D)), axis=-1, keepdims=True))
        g = _rb(jax.nn.sigmoid(logit))
        b = _rb(acc_ref[rows, :])
        obuf[step % 2, rows, :] = g * a + _rb(_rb(1.0 - g) * b)
        o_copy(step, hf).start()

    @pl.when(step == NB - 1)
    def _():
        for hf in range(NH):
            if NB >= 2:
                o_copy(step - 1, hf).wait()
            o_copy(step, hf).wait()


@jax.jit
def pallas_gated_mix__ssm_conv_s5__glu_gated_geglu__prompt_kernel(
    A_x, A_Lambda_re, A_Lambda_im, A_B_re, A_B_im, A_C_re, A_C_im, A_log_dt,
    A_Dskip, B_x, B_w_gate, B_w_up, B_w_down, gate_w,
):
    Bsz, S, D = A_x.shape
    P = A_Lambda_re.shape[0]
    Df = B_w_gate.shape[1]
    assert Bsz == 1 and S % TM == 0 and Df % FC == 0
    NC = Df // FC
    NB = S // TM
    assert NC == NS and NQ == NC

    vec_spec = lambda n: pl.BlockSpec((n,), lambda i: (0,))
    any_spec = pl.BlockSpec(memory_space=pl.ANY)

    out = pl.pallas_call(
        functools.partial(_kernel, P=P, D=D, NC=NC, NB=NB),
        grid=(NB,),
        in_specs=[pl.BlockSpec((TM, D), lambda i: (i, 0)),
                  vec_spec(P), vec_spec(P), vec_spec(P), vec_spec(D), vec_spec(D)]
                 + [any_spec] * 7,
        out_specs=any_spec,
        out_shape=jax.ShapeDtypeStruct((S, D), F32),
        scratch_shapes=[
            pltpu.VMEM((2 * P, D), BF16),
            pltpu.VMEM((D, 2 * P), BF16),
            pltpu.VMEM((NC, D, FC), BF16),
            pltpu.VMEM((NC, D, FC), BF16),
            pltpu.VMEM((NC, FC, D), BF16),
            pltpu.SemaphoreType.DMA((2 + 3 * NC,)),
            pltpu.SemaphoreType.DMA((2 * NQ,)),
            pltpu.SemaphoreType.DMA((2 * NH,)),
            pltpu.VMEM((TM, 2 * P), F32),
            pltpu.VMEM((10, 8, P), F32),
            pltpu.VMEM((8, 2 * P), F32),
            pltpu.VMEM((TM, D), F32),
            pltpu.VMEM((2, TM, D), F32),
        ],
        compiler_params=pltpu.CompilerParams(
            dimension_semantics=("arbitrary",),
            vmem_limit_bytes=100 * 1024 * 1024,
        ),
    )(A_x.reshape(S, D), A_Lambda_re, A_Lambda_im, A_log_dt, A_Dskip, gate_w,
      A_B_re, A_B_im, A_C_re, A_C_im, B_w_gate, B_w_up, B_w_down)
    return out.reshape(Bsz, S, D)
```
